```python
import os as _os
_os.environ.setdefault('JAX_PLATFORMS', 'cpu')
import jax
import jax.numpy as jnp

def _softmax(x, axis=-1):
    return jax.nn.softmax(x, axis=axis)

def _gelu(x):
    return jax.nn.gelu(x, approximate=True)

def _silu(x):
    return jax.nn.silu(x)

def _sigmoid(x):
    return jax.nn.sigmoid(x)

def _layernorm(x, axis=-1, eps=1e-05):
    m = jnp.mean(x, axis=axis, keepdims=True)
    v = jnp.var(x, axis=axis, keepdims=True)
    return (x - m) / jnp.sqrt(v + eps)

def _scatter_add(tgt, idx, src, axis=0):
    return tgt.at[idx].add(src)

def _segment_sum(src, seg, n):
    return jax.ops.segment_sum(src, seg, n)

class _Rng:

    def __init__(self, key):
        self._k = key

    def _next(self):
        self._k, sub = jax.random.split(self._k)
        return sub

    def normal(self, shape):
        return jax.random.normal(self._next(), shape, dtype=jnp.bfloat16)

    def randint(self, lo, hi, shape):
        return jax.random.randint(self._next(), shape, lo, hi, dtype=jnp.int32)

    def uniform(self, shape, lo=0.0, hi=1.0):
        return jax.random.uniform(self._next(), shape, jnp.bfloat16, lo, hi)

    def permutation(self, n):
        return jax.random.permutation(self._next(), n)
kernel_name = 'standalone__autoregressive_conv_wavenet__speech'

def setup_inputs():
    _rng = _Rng(jax.random.key(int.from_bytes(__import__("os").urandom(4), "little")))
    _w = lambda a: (lambda t: t.astype(jnp.bfloat16) if jnp.issubdtype(t.dtype, jnp.floating) else t)(jnp.asarray(a))
    B, T, D, K = (2, 4000, 512, 31)
    return {'x': _w((lambda *s: _rng.normal(s) * 0.05)(B, T, D)), 'w': _w((lambda *s: _rng.normal(s) * 0.05)(K, D, 2 * D)), 'w_o': _w((lambda *s: _rng.normal(s) * 0.05)(D, D))}

def reference(x, w, w_o):
    B, T, D = x.shape
    K = w.shape[0]
    dil = 2
    pad = (K - 1) * dil
    xp = jnp.pad(x, ((0, 0), (pad, 0), (0, 0)))
    h = jnp.einsum('btc,cd->btd', xp[:, pad:pad + T, :], w[0])
    for i in range(1, K):
        off = pad - i * dil
        h = h + jnp.einsum('btc,cd->btd', xp[:, off:off + T, :], w[i])
    f = h[..., :D].copy()
    g = h[..., D:].copy()
    z = jnp.tanh(f) * _sigmoid(g)
    return z @ w_o
```

```python
import functools

import jax
import jax.numpy as jnp
import jax.experimental.pallas as pl
import jax.experimental.pallas.tpu as pltpu


_DIL = 2
_TM = 800
_HALO = 64


def _kernel(x_ref, w_ref, wo_ref, o_ref, xbuf_ref, *, K, D, TM):
    j = pl.program_id(1)
    t0 = pl.multiple_of(j * TM, 16)

    @pl.when(j == 0)
    def _():
        xbuf_ref[0:_HALO, :] = jnp.zeros((_HALO, D), xbuf_ref.dtype)

    @pl.when(j > 0)
    def _():
        xbuf_ref[0:_HALO, :] = x_ref[0, pl.ds(t0 - _HALO, _HALO), :]

    xbuf_ref[_HALO:_HALO + TM, :] = x_ref[0, pl.ds(t0, TM), :]

    h = jnp.zeros((TM, 2 * D), jnp.float32)
    for i in range(K):
        off = _HALO - i * _DIL
        xs = xbuf_ref[off:off + TM, :]
        h = h + jnp.dot(xs, w_ref[i], preferred_element_type=jnp.float32)

    f = h[:, :D]
    g = h[:, D:]
    z = jnp.tanh(f) * jax.nn.sigmoid(g)
    o_ref[0] = jnp.dot(z.astype(jnp.bfloat16), wo_ref[...],
                       preferred_element_type=jnp.float32).astype(o_ref.dtype)


@jax.jit
def pallas_standalone__autoregressive_conv_wavenet__speech_kernel(
    x: jax.Array,
    w: jax.Array,
    w_o: jax.Array,
):
    B, T, D = x.shape
    K = w.shape[0]
    TM = _TM
    assert T % TM == 0 and (K - 1) * _DIL <= _HALO

    kernel = functools.partial(_kernel, K=K, D=D, TM=TM)
    grid_spec = pltpu.PrefetchScalarGridSpec(
        num_scalar_prefetch=0,
        grid=(B, T // TM),
        in_specs=[
            pl.BlockSpec((1, T, D), lambda b, j: (b, 0, 0)),
            pl.BlockSpec((K, D, 2 * D), lambda b, j: (0, 0, 0),
                         pipeline_mode=pl.Buffered(1)),
            pl.BlockSpec((D, D), lambda b, j: (0, 0),
                         pipeline_mode=pl.Buffered(1)),
        ],
        out_specs=pl.BlockSpec((1, TM, D), lambda b, j: (b, j, 0)),
        scratch_shapes=[pltpu.VMEM((TM + _HALO, D), x.dtype)],
    )
    return pl.pallas_call(
        kernel,
        grid_spec=grid_spec,
        out_shape=jax.ShapeDtypeStruct((B, T, D), x.dtype),
        compiler_params=pltpu.CompilerParams(
            dimension_semantics=("arbitrary", "arbitrary"),
            vmem_limit_bytes=100 * 1024 * 1024,
        ),
    )(x, w, w_o)
```

```python
import functools

import jax
import jax.numpy as jnp
from jax import lax
import jax.experimental.pallas as pl
import jax.experimental.pallas.tpu as pltpu


_DIL = 2
_TM = 160
_GRP = 8
_HALO = 64


def _kernel(xc_ref, xp_ref, w_hbm, wo_hbm, o_ref, w_vmem, wo_vmem, xbuf_ref, acc_ref,
            sems, *, K, D, TM):
    b = pl.program_id(0)
    j = pl.program_id(1)
    first = jnp.logical_and(b == 0, j == 0)
    G = pl.cdiv(K, _GRP)
    span = _GRP * _DIL

    def w_copy(i):
        return pltpu.make_async_copy(w_hbm.at[i], w_vmem.at[i], sems.at[i])

    def wo_copy():
        return pltpu.make_async_copy(wo_hbm, wo_vmem, sems.at[K])

    def dot(a, bmat):
        return jnp.dot(a, bmat, preferred_element_type=jnp.float32)

    halo = xp_ref[0, TM - _HALO:TM, :]
    xbuf_ref[0:_HALO, :] = jnp.where(j > 0, halo, jnp.zeros_like(halo))
    xbuf_ref[_HALO:_HALO + TM, :] = xc_ref[0]

    def epilogue(h):
        z = jnp.tanh(h[:, :D]) * jax.nn.sigmoid(h[:, D:])
        o_ref[0] = dot(z.astype(jnp.bfloat16), wo_vmem[...]).astype(o_ref.dtype)

    @pl.when(first)
    def _():
        for i in range(K):
            w_copy(i).start()
        wo_copy().start()
        acc_ref[...] = jnp.zeros_like(acc_ref)

        def group(a, carry):
            base = pl.multiple_of(_HALO - span - span * a, span)
            xg = xbuf_ref[pl.ds(base, TM + span), :]
            n_sure = K - _GRP * (G - 1)
            h = acc_ref[...]
            for r in range(n_sure):
                i = _GRP * a + r
                w_copy(i).wait()
                lo = span - _DIL * r
                h = h + dot(xg[lo:lo + TM], w_vmem[i])
            acc_ref[...] = h
            for r in range(n_sure, _GRP):
                @pl.when(a < G - 1)
                def _():
                    i = _GRP * a + r
                    w_copy(i).wait()
                    lo = span - _DIL * r
                    acc_ref[...] += dot(xg[lo:lo + TM], w_vmem[i])
            return carry

        lax.fori_loop(0, G, group, 0)
        wo_copy().wait()
        epilogue(acc_ref[...])

    @pl.when(jnp.logical_not(first))
    def _():
        h = jnp.zeros((TM, 2 * D), jnp.float32)
        for i in range(K):
            off = _HALO - i * _DIL
            h = h + dot(xbuf_ref[off:off + TM, :], w_vmem[i])
        epilogue(h)


@jax.jit
def pallas_standalone__autoregressive_conv_wavenet__speech_kernel(
    x: jax.Array,
    w: jax.Array,
    w_o: jax.Array,
):
    B, T, D = x.shape
    K = w.shape[0]
    TM = _TM
    assert T % TM == 0 and _HALO <= TM
    assert _GRP * _DIL * pl.cdiv(K, _GRP) <= _HALO and (K - 1) * _DIL <= _HALO

    kernel = functools.partial(_kernel, K=K, D=D, TM=TM)
    grid_spec = pltpu.PrefetchScalarGridSpec(
        num_scalar_prefetch=0,
        grid=(B, T // TM),
        in_specs=[
            pl.BlockSpec((1, TM, D), lambda b, j: (b, j, 0)),
            pl.BlockSpec((1, TM, D), lambda b, j: (b, jnp.maximum(j - 1, 0), 0)),
            pl.BlockSpec(memory_space=pl.ANY),
            pl.BlockSpec(memory_space=pl.ANY),
        ],
        out_specs=pl.BlockSpec((1, TM, D), lambda b, j: (b, j, 0)),
        scratch_shapes=[
            pltpu.VMEM((K, D, 2 * D), w.dtype),
            pltpu.VMEM((D, D), w_o.dtype),
            pltpu.VMEM((TM + _HALO, D), x.dtype),
            pltpu.VMEM((TM, 2 * D), jnp.float32),
            pltpu.SemaphoreType.DMA((K + 1,)),
        ],
    )
    return pl.pallas_call(
        kernel,
        grid_spec=grid_spec,
        out_shape=jax.ShapeDtypeStruct((B, T, D), x.dtype),
        compiler_params=pltpu.CompilerParams(
            dimension_semantics=("arbitrary", "arbitrary"),
            vmem_limit_bytes=100 * 1024 * 1024,
        ),
    )(x, x, w, w_o)
```

```python
import functools

import jax
import jax.numpy as jnp
from jax import lax
import jax.experimental.pallas as pl
import jax.experimental.pallas.tpu as pltpu


_DIL = 2
_TM = 160
_GRP = 8
_HALO = 64


def _kernel(x_ref, x_hbm, w_hbm, wo_hbm, o_ref, w_vmem, wo_vmem, xbuf_ref, xbuf2_ref,
            acc_ref, onext_ref, sems, *, K, D, TM):
    b = pl.program_id(0)
    j = pl.program_id(1)
    first = jnp.logical_and(b == 0, j == 0)
    second = jnp.logical_and(b == 0, j == 1)
    G = pl.cdiv(K, _GRP)
    span = _GRP * _DIL
    TM2 = 2 * TM

    def w_copy(i):
        return pltpu.make_async_copy(w_hbm.at[i], w_vmem.at[i], sems.at[i])

    def wo_copy():
        return pltpu.make_async_copy(wo_hbm, wo_vmem, sems.at[K])

    def x2_copy():
        return pltpu.make_async_copy(x_hbm.at[0, pl.ds(0, TM2), :],
                                     xbuf2_ref.at[pl.ds(_HALO, TM2), :], sems.at[K + 1])

    def dot(a, bmat):
        return jnp.dot(a, bmat, preferred_element_type=jnp.float32)

    def epilogue(h):
        z = jnp.tanh(h[:, :D]) * jax.nn.sigmoid(h[:, D:])
        return dot(z.astype(jnp.bfloat16), wo_vmem[...]).astype(o_ref.dtype)

    @pl.when(first)
    def _():
        x2_copy().start()
        for i in range(K):
            w_copy(i).start()
        wo_copy().start()
        xbuf2_ref[0:_HALO, :] = jnp.zeros((_HALO, D), xbuf2_ref.dtype)
        acc_ref[...] = jnp.zeros_like(acc_ref)
        x2_copy().wait()

        def group(a, carry):
            base = pl.multiple_of(_HALO - span - span * a, span)
            xg = xbuf2_ref[pl.ds(base, TM2 + span), :]
            n_sure = K - _GRP * (G - 1)
            h = acc_ref[...]
            for r in range(n_sure):
                i = _GRP * a + r
                w_copy(i).wait()
                lo = span - _DIL * r
                h = h + dot(xg[lo:lo + TM2], w_vmem[i])
            acc_ref[...] = h
            for r in range(n_sure, _GRP):
                @pl.when(a < G - 1)
                def _():
                    i = _GRP * a + r
                    w_copy(i).wait()
                    lo = span - _DIL * r
                    acc_ref[...] += dot(xg[lo:lo + TM2], w_vmem[i])
            return carry

        lax.fori_loop(0, G, group, 0)
        wo_copy().wait()
        out = epilogue(acc_ref[...])
        o_ref[0] = out[:TM]
        onext_ref[...] = out[TM:]

    @pl.when(second)
    def _():
        o_ref[0] = onext_ref[...]
        xbuf_ref[TM:TM + _HALO, :] = x_ref[0, TM - _HALO:TM, :]

    @pl.when(jnp.logical_not(jnp.logical_or(first, second)))
    def _():
        halo = xbuf_ref[TM:TM + _HALO, :]
        xc = x_ref[0]
        xbuf_ref[0:_HALO, :] = jnp.where(j > 0, halo, jnp.zeros_like(halo))
        xbuf_ref[_HALO:_HALO + TM, :] = xc
        h = dot(xc, w_vmem[0])
        for i in range(1, K):
            off = _HALO - i * _DIL
            h = h + dot(xbuf_ref[off:off + TM, :], w_vmem[i])
        o_ref[0] = epilogue(h)


@jax.jit
def pallas_standalone__autoregressive_conv_wavenet__speech_kernel(
    x: jax.Array,
    w: jax.Array,
    w_o: jax.Array,
):
    B, T, D = x.shape
    K = w.shape[0]
    TM = _TM
    assert T % TM == 0 and _HALO <= TM and T // TM >= 2
    assert _GRP * _DIL * pl.cdiv(K, _GRP) <= _HALO and (K - 1) * _DIL <= _HALO

    kernel = functools.partial(_kernel, K=K, D=D, TM=TM)
    grid_spec = pltpu.PrefetchScalarGridSpec(
        num_scalar_prefetch=0,
        grid=(B, T // TM),
        in_specs=[
            pl.BlockSpec((1, TM, D), lambda b, j: (b, j, 0)),
            pl.BlockSpec(memory_space=pl.ANY),
            pl.BlockSpec(memory_space=pl.ANY),
            pl.BlockSpec(memory_space=pl.ANY),
        ],
        out_specs=pl.BlockSpec((1, TM, D), lambda b, j: (b, j, 0)),
        scratch_shapes=[
            pltpu.VMEM((K, D, 2 * D), w.dtype),
            pltpu.VMEM((D, D), w_o.dtype),
            pltpu.VMEM((TM + _HALO, D), x.dtype),
            pltpu.VMEM((2 * TM + _HALO, D), x.dtype),
            pltpu.VMEM((2 * TM, 2 * D), jnp.float32),
            pltpu.VMEM((TM, D), x.dtype),
            pltpu.SemaphoreType.DMA((K + 2,)),
        ],
    )
    return pl.pallas_call(
        kernel,
        grid_spec=grid_spec,
        out_shape=jax.ShapeDtypeStruct((B, T, D), x.dtype),
        compiler_params=pltpu.CompilerParams(
            dimension_semantics=("arbitrary", "arbitrary"),
            vmem_limit_bytes=100 * 1024 * 1024,
        ),
    )(x, x, w, w_o)
```
